```python
import jax
import jax.numpy as jnp

def _softmax(x, axis=-1):
    return jax.nn.softmax(x, axis=axis)
def _gelu(x):
    return jax.nn.gelu(x, approximate=True)
def _silu(x):
    return jax.nn.silu(x)
def _sigmoid(x):
    return jax.nn.sigmoid(x)
def _layernorm(x, axis=-1, eps=1e-5):
    m = jnp.mean(x, axis=axis, keepdims=True)
    v = jnp.var(x, axis=axis, keepdims=True)
    return (x - m) / jnp.sqrt(v + eps)
def _scatter_add(tgt, idx, src, axis=0):
    return tgt.at[idx].add(src)
def _segment_sum(src, seg, n):
    return jax.ops.segment_sum(src, seg, n)
class _Rng:
    def __init__(self, key):
        self._k = key
    def _next(self):
        self._k, sub = jax.random.split(self._k)
        return sub
    def normal(self, shape):
        return jax.random.normal(self._next(), shape, dtype=jnp.bfloat16)
    def randint(self, lo, hi, shape):
        return jax.random.randint(self._next(), shape, lo, hi, dtype=jnp.int32)
    def uniform(self, shape, lo=0.0, hi=1.0):
        return jax.random.uniform(self._next(), shape, jnp.bfloat16, lo, hi)
    def permutation(self, n):
        return jax.random.permutation(self._next(), n)


kernel_name = 'gated_mix__ssm_conv_h3__sliding_local_dilated__prompt'

def setup_inputs():
    _rng = _Rng(jax.random.key(int.from_bytes(__import__("os").urandom(4), "little")))
    _w = (lambda a: (lambda t: t.astype(jnp.bfloat16) if jnp.issubdtype(t.dtype, jnp.floating) else t)(jnp.asarray(a)))
    def _A_setup():
        B, S, D = 1, 2048, 640
        ks = 4
        return {
            "q": _w((lambda *s: _rng.normal(s) * 0.05)(B, S, D)),
            "k": _w((lambda *s: _rng.normal(s) * 0.05)(B, S, D)),
            "v": _w((lambda *s: _rng.normal(s) * 0.05)(B, S, D)),
            "shift_k": _w((lambda *s: _rng.normal(s) * 0.05)(D, ks) * 0.5),
            "ssm_k": _w((lambda *s: _rng.normal(s) * 0.05)(D, S) * (1.0 / S ** 0.5)),
            "ssm_D": _w((lambda *s: _rng.normal(s) * 0.05)(D)),
        }
    _A_in = _A_setup()

    def _B_setup():
        B, S, D = 1, 2048, 640
        return {
            "x": _w((lambda *s: _rng.normal(s) * 0.05)(B, S, D)),
            "wqkv": _w((lambda *s: _rng.normal(s) * 0.05)(D, 3 * D)),
            "wo": _w((lambda *s: _rng.normal(s) * 0.05)(D, D)),
        }
    _B_in = _B_setup()

    return {
        "A_q": _A_in["q"],
        "A_k": _A_in["k"],
        "A_v": _A_in["v"],
        "A_shift_k": _A_in["shift_k"],
        "A_ssm_k": _A_in["ssm_k"],
        "A_ssm_D": _A_in["ssm_D"],
        "B_x": _B_in["x"],
        "B_wqkv": _B_in["wqkv"],
        "B_wo": _B_in["wo"],
        "gate_w": _w((lambda *s: _rng.normal(s) * 0.05)(640)),
    }

def reference(A_q, A_k, A_v, A_shift_k, A_ssm_k, A_ssm_D, B_x, B_wqkv, B_wo, gate_w):
    def _A_ref(q, k, v, shift_k, ssm_k, ssm_D):
        B, S, D = q.shape
        ks = shift_k.shape[-1]
        k_pad = jnp.pad(k, ((0, 0), (ks - 1, 0), (0, 0)))
        k_shift = jnp.zeros_like(k)
        for t in range(ks):
            k_shift = k_shift + k_pad[:, t:t + S, :] * shift_k[:, ks - 1 - t][None, None, :]
        kv = k_shift * v
        L = 2 * S
        kv_pad = jnp.pad(kv, ((0, 0), (0, S), (0, 0)))
        kf_pad = jnp.pad(ssm_k, ((0, 0), (0, S)))
        kv_f = (lambda x, axes=(-2,-1): jnp.fft.rfft2(x.astype(jnp.float32), axes=axes))(kv_pad[:, None, :, :], axes=(1, 2))
        kf_f = (lambda x, axes=(-2,-1): jnp.fft.rfft2(x.astype(jnp.float32), axes=axes))(kf_pad[:, None, :], axes=(1, 2))
        kf_f = (lambda x, *d: x.transpose(*d))(kf_f, 1, 2, 0)
        y_f = kv_f * kf_f[None, :, :, :]
        y = (lambda x, s, axes=(-2,-1): jnp.fft.irfft2(x, s=s, axes=axes).astype(jnp.bfloat16))(y_f, (1, L), axes=(1, 2))[:, 0, :S, :]
        y = y + kv * ssm_D[None, None, :]
        return q * y

    def _B_ref(x, wqkv, wo):
        B, S, D = x.shape
        H = 32; Dh = D // H
        W, dil = 8, 2
        qkv = (lambda x, *d: x.transpose(*d))((x @ wqkv).reshape(B, S, 3, H, Dh), 2, 0, 3, 1, 4)
        q, k, v = qkv[0], qkv[1], qkv[2]
        scale = Dh ** -0.5
        pos = jnp.arange(S)
        off = jnp.arange(W) * dil
        idx = pos[:, None] - off[None, :]
        mask = idx >= 0
        idx_c = jnp.where(mask, idx, 0).reshape(-1)
        kg = k[:, :, idx_c, :].reshape(B, H, S, W, Dh)
        vg = v[:, :, idx_c, :].reshape(B, H, S, W, Dh)
        logits = jnp.einsum("bhsd,bhswd->bhsw", q, kg) * scale
        logits = jnp.where(mask[None, None, :, :], logits, -1e9)
        attn = _softmax(logits, axis=-1)
        o = jnp.einsum("bhsw,bhswd->bhsd", attn, vg)
        return (lambda x, *d: x.transpose(*d))(o, 0, 2, 1, 3).reshape(B, S, D) @ wo

    x = A_q
    g = _sigmoid((x * gate_w).sum(-1, keepdims=True))
    a = _A_ref(x, A_k, A_v, A_shift_k, A_ssm_k, A_ssm_D)
    b = _B_ref(x, B_wqkv, B_wo)
    return g * a + (1 - g) * b
```

```python
import numpy as np

import jax
import jax.numpy as jnp
import jax.experimental.pallas as pl
import jax.experimental.pallas.tpu as pltpu

S, D = 2048, 640
H, DH = 32, 20
WIN, DIL = 8, 2
KS = 4
LANES = 128
NG = D // LANES
C = 128
NB = S // C
NR = C // 8
HALO = 16
CHALO = 8

TB = 256
SUB = 32

_F32, _BF16 = jnp.float32, jnp.bfloat16
_NT = (((1,), (1,)), ((), ()))


def _dft_matrices():
    g = np.arange(C)[:, None].astype(np.float64)
    n = np.arange(C)[None, :].astype(np.float64)
    ang = np.pi * ((4 * g + 1) * n % (4 * C)) / (2 * C)
    re, im = np.cos(ang), -np.sin(ang)
    fwd = np.stack([re.reshape(NR, 8, C), im.reshape(NR, 8, C)], axis=1).reshape(2 * C, C)
    return fwd.astype(np.float32), (fwd.T / C).astype(np.float32)


_FWD, _INV = _dft_matrices()


def _cols(c):
    return slice(c * LANES, (c + 1) * LANES)


def _toeplitz(x, h):
    out = []
    for i in range(len(x)):
        acc = x[0] * h[i]
        for j in range(1, i + 1):
            acc = acc + x[j] * h[i - j]
        out.append(acc)
    return out


def _kernel(x_hbm, k_hbm, v_hbm, sk_ref, h_hbm, d_ref, w_hbm, wo_hbm, gw_ref, fwd_ref, inv_ref,
            o_hbm,
            xs, ks, vs, hs, ws, wos, wt32, wo32, wp, wop, qbuf, kbuf, vbuf, obuf, kf,
            kvh, hh, zb, bb, gq, ob, sem_in, sem_out):
    def col_copy(src, dst, n, sem0):
        return [pltpu.make_async_copy(src.at[:, _cols(c)], dst.at[c], sem_in.at[sem0 + c])
                for c in range(n)]

    cp_w = col_copy(w_hbm, ws, 3 * NG, 0)
    cp_x = col_copy(x_hbm, xs, NG, 15)
    cp_wo = col_copy(wo_hbm, wos, NG, 20)
    cp_h = col_copy(h_hbm, hs, NB, 25)
    cp_k = col_copy(k_hbm, ks, NG, 41)
    cp_v = col_copy(v_hbm, vs, NG, 46)
    for cp in cp_h + cp_k + cp_v + cp_w + cp_x + cp_wo:
        cp.start()

    taps = sk_ref[...].astype(_F32).T
    dvec = d_ref[...].astype(_F32)
    gvec = gw_ref[...].astype(_F32)
    for c in range(NG):
        kbuf[c, 0:HALO, :] = jnp.zeros((HALO, LANES), _F32)
        vbuf[c, 0:HALO, :] = jnp.zeros((HALO, LANES), _F32)
        kf[c, 0:CHALO, :] = jnp.zeros((CHALO, LANES), _F32)

    def fwd_h(m):
        r = jax.lax.dot_general(fwd_ref[...], hs[m], _NT, preferred_element_type=_F32)
        for c in range(NG):
            hh[c, m] = r[:, _cols(c)]

    def fwd_kv(j):
        t0 = pl.multiple_of(j * C, C)
        kvs = []
        for c in range(NG):
            k0 = ks[c, pl.ds(t0, C), :].astype(_F32)
            kf[c, pl.ds(t0 + CHALO, C), :] = k0
            acc = k0 * taps[0:1, _cols(c)]
            for t in range(1, KS):
                acc = acc + kf[c, pl.ds(t0 + (CHALO - t), C), :] * taps[t:t + 1, _cols(c)]
            kvs.append((acc * vs[c, pl.ds(t0, C), :].astype(_F32)).astype(_BF16))
        r = jnp.dot(fwd_ref[...], jnp.concatenate(kvs, axis=1), preferred_element_type=_F32)
        for c in range(NG):
            kvh[c, j] = r[:, _cols(c)]

    def transpose_w(n):
        t = ws[n].astype(_F32).T
        for c in range(NG):
            wt32[c, n * LANES:(n + 1) * LANES, :] = t[:, _cols(c)]

    def permute_w(p):
        for c in range(NG):
            for d in range(DH):
                wp[c, p * D + d * H:p * D + (d + 1) * H, :] = (
                    wt32[c, pl.ds(p * D + d, H, stride=DH), :].astype(_BF16))

    def permute_wo(c):
        wo32[c] = wos[c].astype(_F32)
        for d in range(DH):
            wop[c, d * H:(d + 1) * H, :] = wo32[c, pl.ds(d, H, stride=DH), :].astype(_BF16)

    def block_conv(c, r):
        re = pl.ds(pl.multiple_of(r * 16, 16), 8)
        im = pl.ds(pl.multiple_of(r * 16 + 8, 8), 8)
        hr = [hh[c, m, re, :] for m in range(NB)]
        hi = [hh[c, m, im, :] for m in range(NB)]
        hr, hi = ([hr[0]] + [hr[m] - hi[m - 1] for m in range(1, NB)],
                  [hi[0]] + [hi[m] + hr[m - 1] for m in range(1, NB)])
        a = [kvh[c, j, re, :] for j in range(NB)]
        b = [kvh[c, j, im, :] for j in range(NB)]
        k1 = _toeplitz([a[j] + b[j] for j in range(NB)], hr)
        k3 = _toeplitz(b, [hr[m] + hi[m] for m in range(NB)])
        zr = [k1[i] - k3[i] for i in range(NB)]
        k2 = _toeplitz(a, [hi[m] - hr[m] for m in range(NB)])
        for i in range(NB):
            z = jnp.concatenate([zr[i], k1[i] + k2[i]], axis=0)
            zb[c, i, pl.ds(pl.multiple_of(r * 16, 16), 16), :] = z.astype(_BF16)

    scale = DH ** -0.5

    def attention_block(i):
        t0 = pl.multiple_of(i * TB, TB)
        xb = jnp.concatenate([xs[c, pl.ds(t0, TB), :] for c in range(NG)], axis=1)

        def proj(p):
            w = jnp.concatenate([wp[c, p * D:(p + 1) * D, :] for c in range(NG)], axis=1)
            return jax.lax.dot_general(xb, w, _NT, preferred_element_type=_F32)

        r = proj(1)
        for c in range(NG):
            kbuf[c, pl.ds(t0 + HALO, TB), :] = r[:, _cols(c)]
        r = proj(0)
        for c in range(NG):
            qbuf[c] = r[:, _cols(c)]
        r = proj(2)
        for c in range(NG):
            vbuf[c, pl.ds(t0 + HALO, TB), :] = r[:, _cols(c)]

        omg = []
        for u in range(TB // SUB):
            r0 = t0 + u * SUB
            row = r0 + jax.lax.broadcasted_iota(jnp.int32, (SUB, LANES), 0)
            q = [qbuf[c, u * SUB:(u + 1) * SUB, :] for c in range(NG)]
            logits = []
            for w in range(WIN):
                rows = pl.ds(r0 + (HALO - DIL * w), SUB)
                p = q[0] * kbuf[0, rows, :]
                for c in range(1, NG):
                    p = p + q[c] * kbuf[c, rows, :]
                p = p + pltpu.roll(p, 2 * H, 1)
                p = p + pltpu.roll(p, H, 1)
                if w:
                    p = jnp.where(row >= DIL * w, p, -1e9 / scale)
                logits.append(p)
            m = logits[0]
            for w in range(1, WIN):
                m = jnp.maximum(m, logits[w])
            e = [jnp.exp2((l - m) * (scale * np.log2(np.e))) for l in logits]
            den = e[0]
            for w in range(1, WIN):
                den = den + e[w]
            rden = 1.0 / den
            for c in range(NG):
                acc = e[0] * vbuf[c, pl.ds(r0 + HALO, SUB), :]
                for w in range(1, WIN):
                    acc = acc + e[w] * vbuf[c, pl.ds(r0 + (HALO - DIL * w), SUB), :]
                obuf[c, u * SUB:(u + 1) * SUB, :] = (acc * rden).astype(_BF16)
            xf = [xs[c, pl.ds(r0, SUB), :].astype(_F32) for c in range(NG)]
            gs = xf[0] * gvec[:, _cols(0)]
            for c in range(1, NG):
                gs = gs + xf[c] * gvec[:, _cols(c)]
            g = jax.nn.sigmoid(jnp.sum(gs, axis=1, keepdims=True))
            for c in range(NG):
                gq[c, pl.ds(r0, SUB), :] = g * xf[c]
            omg.append(1.0 - g)

        o = jnp.concatenate([obuf[c] for c in range(NG)], axis=1)
        wo = jnp.concatenate([wop[c] for c in range(NG)], axis=1)
        b = jnp.dot(o, wo, preferred_element_type=_F32) * jnp.concatenate(omg, axis=0)
        for c in range(NG):
            bb[c, pl.ds(t0, TB), :] = b[:, _cols(c)]

    def out_copy(i, c):
        rows = pl.ds(pl.multiple_of(i * C, C), C)
        return pltpu.make_async_copy(ob.at[c, rows, :], o_hbm.at[rows, _cols(c)],
                                     sem_out.at[i * NG + c])

    def finish(i):
        rows = pl.ds(pl.multiple_of(i * C, C), C)
        z = jnp.concatenate([zb[c, i] for c in range(NG)], axis=1)
        y = jnp.dot(inv_ref[...], z, preferred_element_type=_F32)
        for c in range(NG):
            ob[c, rows, :] = (gq[c, rows, :] * y[:, _cols(c)] + bb[c, rows, :]).astype(_BF16)
        for c in range(NG):
            out_copy(i, c).start()

    def loop(n, unroll, body):
        def step(s, carry):
            for u in range(unroll):
                body(s * unroll + u)
            return carry
        jax.lax.fori_loop(0, n // unroll, step, 0)

    for cp in cp_h:
        cp.wait()
    loop(NB, 4, fwd_h)
    for c in range(NG):
        for r in range(NR):
            hh[c, 0, r * 16:r * 16 + 8, :] = hh[c, 0, r * 16:r * 16 + 8, :] + dvec[:, _cols(c)]
    for cp in cp_k + cp_v:
        cp.wait()
    loop(NB, 4, fwd_kv)
    for p in range(3):
        for n in range(p * NG, (p + 1) * NG):
            cp_w[n].wait()
            transpose_w(n)
        permute_w(p)
    for c in range(NG):
        cp_wo[c].wait()
        permute_wo(c)
    for cp in cp_x:
        cp.wait()

    nstep = S // TB
    per = NR // nstep

    def main(i):
        attention_block(i)
        for u in range(per):
            for c in range(NG):
                block_conv(c, i * per + u)

    loop(nstep, 1, main)
    loop(NB, 4, finish)
    for i in range(NB):
        for c in range(NG):
            out_copy(i, c).wait()


@jax.jit
def pallas_gated_mix__ssm_conv_h3__sliding_local_dilated__prompt_kernel(
    A_q: jax.Array,
    A_k: jax.Array,
    A_v: jax.Array,
    A_shift_k: jax.Array,
    A_ssm_k: jax.Array,
    A_ssm_D: jax.Array,
    B_x: jax.Array,
    B_wqkv: jax.Array,
    B_wo: jax.Array,
    gate_w: jax.Array,
):
    del B_x
    hbm = pl.BlockSpec(memory_space=pl.ANY)
    vmem = pl.BlockSpec(memory_space=pltpu.VMEM)
    V = pltpu.VMEM
    out = pl.pallas_call(
        _kernel,
        out_shape=jax.ShapeDtypeStruct((S, D), _BF16),
        in_specs=[hbm, hbm, hbm, vmem, hbm, vmem, hbm, hbm, vmem, vmem, vmem],
        out_specs=hbm,
        scratch_shapes=[
            V((NG, S, LANES), _BF16),
            V((NG, S, LANES), _BF16),
            V((NG, S, LANES), _BF16),
            V((NB, D, LANES), _BF16),
            V((3 * NG, D, LANES), _BF16),
            V((NG, D, LANES), _BF16),
            V((NG, 3 * D, LANES), _F32),
            V((NG, D, LANES), _F32),
            V((NG, 3 * D, LANES), _BF16),
            V((NG, D, LANES), _BF16),
            V((NG, TB, LANES), _F32),
            V((NG, HALO + S, LANES), _F32),
            V((NG, HALO + S, LANES), _F32),
            V((NG, TB, LANES), _BF16),
            V((NG, CHALO + S, LANES), _F32),
            V((NG, NB, 2 * C, LANES), _F32),
            V((NG, NB, 2 * C, LANES), _F32),
            V((NG, NB, 2 * C, LANES), _BF16),
            V((NG, S, LANES), _F32),
            V((NG, S, LANES), _F32),
            V((NG, S, LANES), _BF16),
            pltpu.SemaphoreType.DMA((51,)),
            pltpu.SemaphoreType.DMA((NB * NG,)),
        ],
        compiler_params=pltpu.CompilerParams(vmem_limit_bytes=100 * 2**20),
    )(
        A_q.reshape(S, D), A_k.reshape(S, D), A_v.reshape(S, D), A_shift_k, A_ssm_k,
        A_ssm_D.reshape(1, D), B_wqkv, B_wo, gate_w.reshape(1, D),
        jnp.asarray(_FWD, _BF16), jnp.asarray(_INV, _BF16),
    )
    return out.reshape(1, S, D)
```

```python
import numpy as np

import jax
import jax.numpy as jnp
import jax.experimental.pallas as pl
import jax.experimental.pallas.tpu as pltpu

S, D = 2048, 640
H, DH = 32, 20
WIN, DIL = 8, 2
KS = 4
LANES = 128
NG = D // LANES
C = 128
NB = S // C
NR = C // 8
HALO = 16
CHALO = 8

TB = 256
SUB = 16
NCAT = 4
NQ = NB // NCAT
TILE = 4
PACE = 4

_F32, _BF16, _U32 = jnp.float32, jnp.bfloat16, jnp.uint32
_NT = (((1,), (1,)), ((), ()))


def _dft_matrices():
    g = np.arange(C)[:, None].astype(np.float64)
    n = np.arange(C)[None, :].astype(np.float64)
    ang = np.pi * ((4 * g + 1) * n % (4 * C)) / (2 * C)
    re, im = np.cos(ang), -np.sin(ang)
    fwd = np.stack([re.reshape(NR, 8, C), im.reshape(NR, 8, C)], axis=1).reshape(2 * C, C)
    return fwd.astype(np.float32), (fwd.T / C).astype(np.float32)


_FWD, _INV = _dft_matrices()


def _cols(c):
    return slice(c * LANES, (c + 1) * LANES)


def _pack(x):
    return pltpu.bitcast(x.astype(_BF16), _U32)


def _unpack(x):
    return pltpu.bitcast(x, _BF16)


def _tree(op, xs):
    while len(xs) > 1:
        xs = [op(xs[i], xs[i + 1]) for i in range(0, len(xs), 2)]
    return xs[0]


def _kernel(x_hbm, k_hbm, v_hbm, sk_ref, h_hbm, d_ref, w_hbm, wo_hbm, gw_ref, fwd_ref, inv_ref,
            o_hbm,
            xs, ks, vs, hs, ws, wos, wt32, wp, qkv, obuf, kf,
            small, yb, ob, zb, spec, sem_in, sem_out):
    def copy(src, dst, idx, sem):
        return pltpu.make_async_copy(src.at[idx], dst.at[idx], sem_in.at[sem])

    def h_copy(c):
        return copy(h_hbm, hs, (pl.ds(pl.multiple_of(c * LANES, LANES), LANES), slice(None)), c)

    def kv_copies(q):
        rows = (pl.ds(pl.multiple_of(q * NCAT * C, NCAT * C), NCAT * C), slice(None))
        return [copy(k_hbm, ks, rows, NG + 2 * q), copy(v_hbm, vs, rows, NG + 2 * q + 1)]

    sem0 = NG + 2 * NQ

    def w_copy(p):
        return copy(w_hbm, ws, (slice(None), pl.ds(pl.multiple_of(p * D, LANES), D)), sem0 + p)

    cp_x = [copy(x_hbm, xs, (pl.ds(0, 2 * TB), slice(None)), sem0 + 3),
            copy(x_hbm, xs, (pl.ds(2 * TB, S - 2 * TB), slice(None)), sem0 + 4)]
    cp_wo = copy(wo_hbm, wos, (slice(None), slice(None)), sem0 + 5)
    for cp in ([h_copy(c) for c in range(NG)] + [w_copy(p) for p in range(3)] + [cp_x[0]]
               + sum([kv_copies(q) for q in range(NQ)], []) + [cp_x[1], cp_wo]):
        cp.start()

    taps = sk_ref[...].astype(_F32)
    dvec = d_ref[...].astype(_F32)
    gvec = gw_ref[...].astype(_F32)
    for c in range(NG):
        qkv[NG + c, 0:HALO, :] = jnp.zeros((HALO, LANES), _F32)
        qkv[2 * NG + c, 0:HALO, :] = jnp.zeros((HALO, LANES), _F32)
        small[c, 0:KS, :] = taps[:, _cols(c)]
        small[c, KS:KS + 1, :] = dvec[c:c + 1, :]
        kf[c, 0:CHALO, :] = jnp.zeros((CHALO, LANES), _F32)

    for c in range(2):
        wp[NG, (c + 1) * C // 2:(c + 2) * C // 2, :] = pltpu.bitcast(inv_ref[:, _cols(c)], _U32)

    wp[NG, 2 * C:3 * C, :] = pltpu.bitcast(fwd_ref[...], _U32)

    def fwd_matrix():
        return _unpack(wp[NG, 2 * C:3 * C, :])

    def forward_h(c, q):
        b0 = q * NCAT
        hb = jnp.concatenate([hs[pl.ds(pl.multiple_of(c * LANES, LANES), LANES), _cols(b0 + u)] for u in range(NCAT)], axis=0)
        r = jax.lax.dot_general(fwd_matrix(), hb, _NT, preferred_element_type=_F32)
        dv = small[c, KS:KS + 1, :]
        for u in range(NCAT):
            for g in range(NR):
                hr, hi = r[g * 16:g * 16 + 8, _cols(u)], r[g * 16 + 8:g * 16 + 16, _cols(u)]
                if b0 + u == 0:
                    hr = hr + dv
                spec[c, NB + b0 + u, g * 24:g * 24 + 8, :] = hr
                spec[c, NB + b0 + u, g * 24 + 8:g * 24 + 16, :] = hr + hi
                spec[c, NB + b0 + u, g * 24 + 16:g * 24 + 24, :] = hi - hr

    def forward_kv(c, q):
        b0 = q * NCAT
        t0 = pl.multiple_of(b0 * C, NCAT * C)
        k0 = ks[pl.ds(t0, NCAT * C), _cols(c)].astype(_F32)
        kf[c, pl.ds(t0 + CHALO, NCAT * C), :] = k0
        acc = k0 * small[c, 0:1, :]
        for t in range(1, KS):
            acc = acc + kf[c, pl.ds(t0 + (CHALO - t), NCAT * C), :] * small[c, t:t + 1, :]
        kv = (acc * vs[pl.ds(t0, NCAT * C), _cols(c)].astype(_F32)).astype(_BF16)
        kv = jnp.concatenate([kv[u * C:(u + 1) * C] for u in range(NCAT)], axis=1)
        r = jnp.dot(fwd_matrix(), kv, preferred_element_type=_F32)
        for u in range(NCAT):
            for g in range(NR):
                a, b = r[g * 16:g * 16 + 8, _cols(u)], r[g * 16 + 8:g * 16 + 16, _cols(u)]
                spec[c, b0 + u, g * 24:g * 24 + 8, :] = a + b
                spec[c, b0 + u, g * 24 + 8:g * 24 + 16, :] = b
                spec[c, b0 + u, g * 24 + 16:g * 24 + 24, :] = a

    def inverse(c, q):
        inv = jnp.concatenate([_unpack(wp[NG, (u + 1) * C // 2:(u + 2) * C // 2, :]) for u in range(2)], axis=1)
        z = jnp.concatenate([_unpack(zb[c, q * NCAT + u]) for u in range(NCAT)], axis=1)
        y = jnp.dot(inv, z, preferred_element_type=_F32)
        for u in range(NCAT):
            yb[c, pl.ds(pl.multiple_of((q * NCAT + u) * C, C), C), :] = y[:, _cols(u)]

    def permute_w(p):
        for n in range(NG):
            t = ws[:, pl.ds(pl.multiple_of(p * D + n * LANES, LANES), LANES)].astype(_F32).T
            for c in range(NG):
                wt32[c, _cols(n), :] = t[:, _cols(c)]
        for c in range(NG):
            for d in range(DH):
                rows = pl.ds(pl.multiple_of(p * (D // 2) + d * (H // 2), H // 2), H // 2)
                wp[c, rows, :] = _pack(wt32[c, pl.ds(d, H, stride=DH), :])

    def permute_wo(c):
        wt32[c] = wos[:, _cols(c)].astype(_F32)
        for d in range(DH):
            wp[c, (3 * D + d * H) // 2:(3 * D + (d + 1) * H) // 2, :] = _pack(wt32[c, pl.ds(d, H, stride=DH), :])

    def block_conv(c, r):
        r24 = pl.multiple_of(r * 24, 8)
        tok = pl.ds(pl.multiple_of(r * 8, 8), 8)
        cnt = 0
        prev = None
        for i0 in range(0, NB, TILE):
            ks = []
            for p in range(3):
                rows = pl.ds(r24 + 8 * p, 8)
                acc = [None] * TILE
                hw = {}
                for j0 in range(0, i0 + TILE, TILE):
                    need = {i - j for i in range(i0, i0 + TILE) for j in range(j0, j0 + TILE) if i >= j}
                    hw = {m: hw[m] if m in hw else spec[c, NB + m, rows, :] for m in sorted(need)}
                    for j in range(j0, j0 + TILE):
                        xj = spec[c, j, rows, :]
                        for i in range(max(i0, j), i0 + TILE):
                            t = xj * hw[i - j]
                            acc[i - i0] = t if acc[i - i0] is None else acc[i - i0] + t
                    cnt += 1
                    if cnt % PACE == 0:
                        for n, v in enumerate(acc):
                            spec[c, 2 * NB, pl.ds(pl.multiple_of(r * 8 + n * C // 2, 8), 8), :] = v
                ks.append(acc)
            for u in range(TILE):
                yr, yi = ks[0][u] - ks[1][u], ks[0][u] + ks[2][u]
                zr, zi = (yr, yi) if prev is None else (yr - prev[1], yi + prev[0])
                prev = yr, yi
                z = jnp.concatenate([zr, zi], axis=0)
                zb[c, i0 + u, tok, :] = _pack(z)

    scale = DH ** -0.5


    def weights(p):
        rows = pl.ds(pl.multiple_of(p * (D // 2), D // 2), D // 2)
        return jnp.concatenate([_unpack(wp[c, rows, :]) for c in range(NG)], axis=1)

    def project(n):
        i, p = n // 3, n % 3
        xb = xs[pl.ds(pl.multiple_of(i * TB, TB), TB), :]
        r = jax.lax.dot_general(xb, weights(p), _NT, preferred_element_type=_F32)
        for c in range(NG):
            qkv[p * NG + c, pl.ds(pl.multiple_of(HALO + i * TB, HALO), TB), :] = r[:, _cols(c)]

    def attend(s, u, masked):
        r0 = pl.multiple_of(HALO + s * TB + u * SUB, SUB)
        q = [qkv[c, pl.ds(r0, SUB), :] for c in range(NG)]
        logits = []
        for w in range(WIN):
            rows = pl.ds(r0 - DIL * w, SUB)
            p = q[0] * qkv[NG, rows, :]
            for c in range(1, NG):
                p = p + q[c] * qkv[NG + c, rows, :]
            logits.append(p)
        logits = [p + pltpu.roll(p, 2 * H, 1) for p in logits]
        yield
        logits = [p + pltpu.roll(p, H, 1) for p in logits]
        yield
        if masked and u * SUB < DIL * (WIN - 1):
            row = u * SUB + jax.lax.broadcasted_iota(jnp.int32, (SUB, LANES), 0)
            logits = [p if w == 0 else jnp.where(row >= DIL * w, p, -1e9 / scale)
                      for w, p in enumerate(logits)]
        m = _tree(jnp.maximum, logits)
        e = [jnp.exp2((l - m) * (scale * np.log2(np.e))) for l in logits]
        rden = 1.0 / _tree(jnp.add, e)
        for c in range(NG):
            acc = e[0] * qkv[2 * NG + c, pl.ds(r0, SUB), :]
            for w in range(1, WIN):
                acc = acc + e[w] * qkv[2 * NG + c, pl.ds(r0 - DIL * w, SUB), :]
            obuf[c, pl.ds(pl.multiple_of(s * (TB // 2) + u * (SUB // 2), SUB // 2), SUB // 2), :] = _pack(acc * rden)
        yield

    def out_copy(i):
        rows = pl.ds(pl.multiple_of(i * TB, TB), TB)
        return pltpu.make_async_copy(ob.at[rows, :], o_hbm.at[rows, :], sem_out.at[i])

    def out_proj(i):
        rows = pl.ds(pl.multiple_of(i * TB, TB), TB)
        half = pl.ds(pl.multiple_of(i * (TB // 2), TB // 2), TB // 2)
        o = jnp.concatenate([_unpack(obuf[c, half, :]) for c in range(NG)], axis=1)
        b = jnp.dot(o, weights(3), preferred_element_type=_F32)
        xf = [xs[rows, _cols(c)].astype(_F32) for c in range(NG)]
        gs = xf[0] * gvec[0:1, :]
        for c in range(1, NG):
            gs = gs + xf[c] * gvec[c:c + 1, :]
        g = jax.nn.sigmoid(jnp.sum(gs, axis=1, keepdims=True))
        for c in range(NG):
            bc = b[:, _cols(c)]
            ob[rows, _cols(c)] = (bc + g * (xf[c] * yb[c, rows, :] - bc)).astype(_BF16)
        out_copy(i).start()

    nstep = S // TB
    npos = NR // NQ

    def attention(s, masked=False):
        n = TB // SUB
        work = [attend(s, u, masked) for u in range(n)]
        next(work[0])
        for u in range(n):
            if u + 1 < n:
                next(work[u + 1])
            next(work[u])
            next(work[u])

    def conv_step(c, q):
        for u in range(npos):
            block_conv(c, q * npos + u)

    @pl.loop(0, NG)
    def _(c):
        h_copy(c).wait()
        for q in range(NQ):
            forward_h(c, q)

    @pl.loop(0, 3)
    def _(p):
        w_copy(p).wait()
        permute_w(p)

    cp_x[0].wait()

    project(0)

    @pl.loop(0, NQ - 1)
    def _(q):
        for cp in kv_copies(q):
            cp.wait()
        project(q + 1)
        for c in range(NG):
            forward_kv(c, q)

    for cp in kv_copies(NQ - 1):
        cp.wait()
    for c in range(NG):
        forward_kv(c, NQ - 1)

    @pl.loop(0, NQ)
    def _(q):
        @pl.when(q == 2)
        def _():
            cp_x[1].wait()
        project(NQ + q)
        conv_step(0, q)

    @pl.loop(NQ, NG * NQ)
    def _(n):
        c, q = n // NQ, n % NQ
        inverse(c - 1, q)
        project(NQ + n)
        conv_step(c, q)

    cp_wo.wait()
    for q in range(NQ):
        inverse(NG - 1, q)
    attention(0, masked=True)
    for c in range(NG):
        permute_wo(c)

    @pl.loop(1, nstep)
    def _(s):
        out_proj(s - 1)
        attention(s)

    out_proj(nstep - 1)
    for i in range(nstep):
        out_copy(i).wait()


@jax.jit
def pallas_gated_mix__ssm_conv_h3__sliding_local_dilated__prompt_kernel(
    A_q: jax.Array,
    A_k: jax.Array,
    A_v: jax.Array,
    A_shift_k: jax.Array,
    A_ssm_k: jax.Array,
    A_ssm_D: jax.Array,
    B_x: jax.Array,
    B_wqkv: jax.Array,
    B_wo: jax.Array,
    gate_w: jax.Array,
):
    del B_x
    hbm = pl.BlockSpec(memory_space=pl.ANY)
    vmem = pl.BlockSpec(memory_space=pltpu.VMEM)
    V = pltpu.VMEM
    out = pl.pallas_call(
        _kernel,
        out_shape=jax.ShapeDtypeStruct((S, D), _BF16),
        in_specs=[hbm, hbm, hbm, vmem, hbm, vmem, hbm, hbm, vmem, vmem, vmem],
        out_specs=hbm,
        scratch_shapes=[
            V((S, D), _BF16),
            V((S, D), _BF16),
            V((S, D), _BF16),
            V((D, S), _BF16),
            V((D, 3 * D), _BF16),
            V((D, D), _BF16),
            V((NG, D, LANES), _F32),
            V((NG + 1, 4 * D // 2, LANES), _U32),
            V((3 * NG, HALO + S, LANES), _F32),
            V((NG, S // 2, LANES), _U32),
            V((NG, CHALO + S, LANES), _F32),
            V((NG, 8, LANES), _F32),
            V((NG, S, LANES), _F32),
            V((S, D), _BF16),
            V((NG, NB, C, LANES), _U32),
            V((NG, 2 * NB + 1, 3 * C, LANES), _F32),
            pltpu.SemaphoreType.DMA((NG + 2 * NQ + 6,)),
            pltpu.SemaphoreType.DMA((S // TB,)),
        ],
        compiler_params=pltpu.CompilerParams(vmem_limit_bytes=112 * 2**20),
    )(
        A_q.reshape(S, D), A_k.reshape(S, D), A_v.reshape(S, D), A_shift_k.T, A_ssm_k,
        A_ssm_D.reshape(NG, LANES), B_wqkv, B_wo, gate_w.reshape(NG, LANES),
        jnp.asarray(_FWD, _BF16), jnp.asarray(_INV, _BF16),
    )
    return out.reshape(1, S, D)
```

```python
import numpy as np

import jax
import jax.numpy as jnp
import jax.experimental.pallas as pl
import jax.experimental.pallas.tpu as pltpu

S, D = 2048, 640
H, DH = 32, 20
WIN, DIL = 8, 2
KS = 4
LANES = 128
NG = D // LANES
C = 128
NB = S // C
NR = C // 8
HALO = 16
CHALO = 8

TB = 256
SUB = 16
NCAT = 4
NQ = NB // NCAT
TILE = 4
PACE = 4

_F32, _BF16, _U32 = jnp.float32, jnp.bfloat16, jnp.uint32
_NT = (((1,), (1,)), ((), ()))


def _dft_matrices():
    g = np.arange(C)[:, None].astype(np.float64)
    n = np.arange(C)[None, :].astype(np.float64)
    ang = np.pi * ((4 * g + 1) * n % (4 * C)) / (2 * C)
    re, im = np.cos(ang), -np.sin(ang)
    fwd = np.stack([re.reshape(NR, 8, C), im.reshape(NR, 8, C)], axis=1).reshape(2 * C, C)
    return fwd.astype(np.float32), (fwd.T / C).astype(np.float32)


_FWD, _INV = _dft_matrices()


def _cols(c):
    return slice(c * LANES, (c + 1) * LANES)


def _pack(x):
    return pltpu.bitcast(x.astype(_BF16), _U32)


def _unpack(x):
    return pltpu.bitcast(x, _BF16)


def _tree(op, xs):
    while len(xs) > 1:
        xs = [op(xs[i], xs[i + 1]) for i in range(0, len(xs), 2)]
    return xs[0]


def _kernel(x_hbm, k_hbm, v_hbm, sk_ref, h_hbm, d_ref, w_hbm, wo_hbm, gw_ref, fwd_ref, inv_ref,
            o_hbm,
            xs, ks, vs, hs, ws, wos, wt32, wp, qkv, obuf, kf,
            small, yb, ob, zb, spec, sem_in, sem_out):
    def copy(src, dst, idx, sem):
        return pltpu.make_async_copy(src.at[idx], dst.at[idx], sem_in.at[sem])

    def h_copy(c):
        return copy(h_hbm, hs, (pl.ds(pl.multiple_of(c * LANES, LANES), LANES), slice(None)), c)

    def kv_copies(q):
        rows = (pl.ds(pl.multiple_of(q * NCAT * C, NCAT * C), NCAT * C), slice(None))
        return [copy(k_hbm, ks, rows, NG + 2 * q), copy(v_hbm, vs, rows, NG + 2 * q + 1)]

    sem0 = NG + 2 * NQ

    def w_copy(p):
        return copy(w_hbm, ws, (slice(None), pl.ds(pl.multiple_of(p * D, LANES), D)), sem0 + p)

    cp_x = [copy(x_hbm, xs, (pl.ds(0, TB), slice(None)), sem0 + 3),
            copy(x_hbm, xs, (pl.ds(TB, TB), slice(None)), sem0 + 6),
            copy(x_hbm, xs, (pl.ds(2 * TB, S - 2 * TB), slice(None)), sem0 + 4)]
    cp_wo = copy(wo_hbm, wos, (slice(None), slice(None)), sem0 + 5)
    for cp in ([h_copy(c) for c in range(NG)] + [w_copy(p) for p in range(3)] + [cp_x[0]]
               + kv_copies(0) + kv_copies(1) + [cp_x[1]] + kv_copies(2) + kv_copies(3) + [cp_x[2], cp_wo]):
        cp.start()

    taps = sk_ref[...].astype(_F32)
    dvec = d_ref[...].astype(_F32)
    gvec = gw_ref[...].astype(_F32)
    for c in range(NG):
        qkv[NG + c, 0:HALO, :] = jnp.zeros((HALO, LANES), _F32)
        qkv[2 * NG + c, 0:HALO, :] = jnp.zeros((HALO, LANES), _F32)
        small[c, 0:KS, :] = taps[:, _cols(c)]
        small[c, KS:KS + 1, :] = dvec[c:c + 1, :]
        kf[c, 0:CHALO, :] = jnp.zeros((CHALO, LANES), _F32)

    for c in range(2):
        wp[NG, (c + 1) * C // 2:(c + 2) * C // 2, :] = pltpu.bitcast(inv_ref[:, _cols(c)], _U32)

    wp[NG, 2 * C:3 * C, :] = pltpu.bitcast(fwd_ref[...], _U32)

    def fwd_matrix():
        return _unpack(wp[NG, 2 * C:3 * C, :])

    def forward_h(c, q):
        b0 = q * NCAT
        hb = jnp.concatenate([hs[pl.ds(pl.multiple_of(c * LANES, LANES), LANES), _cols(b0 + u)] for u in range(NCAT)], axis=0)
        r = jax.lax.dot_general(fwd_matrix(), hb, _NT, preferred_element_type=_F32)
        dv = small[c, KS:KS + 1, :]
        for u in range(NCAT):
            for g in range(NR):
                hr, hi = r[g * 16:g * 16 + 8, _cols(u)], r[g * 16 + 8:g * 16 + 16, _cols(u)]
                if b0 + u == 0:
                    hr = hr + dv
                spec[c, NB + b0 + u, g * 24:g * 24 + 8, :] = hr
                spec[c, NB + b0 + u, g * 24 + 8:g * 24 + 16, :] = hr + hi
                spec[c, NB + b0 + u, g * 24 + 16:g * 24 + 24, :] = hi - hr

    def forward_kv(c, q):
        b0 = q * NCAT
        t0 = pl.multiple_of(b0 * C, NCAT * C)
        k0 = ks[pl.ds(t0, NCAT * C), _cols(c)].astype(_F32)
        kf[c, pl.ds(t0 + CHALO, NCAT * C), :] = k0
        acc = k0 * small[c, 0:1, :]
        for t in range(1, KS):
            acc = acc + kf[c, pl.ds(t0 + (CHALO - t), NCAT * C), :] * small[c, t:t + 1, :]
        kv = (acc * vs[pl.ds(t0, NCAT * C), _cols(c)].astype(_F32)).astype(_BF16)
        kv = jnp.concatenate([kv[u * C:(u + 1) * C] for u in range(NCAT)], axis=1)
        r = jnp.dot(fwd_matrix(), kv, preferred_element_type=_F32)
        for u in range(NCAT):
            for g in range(NR):
                a, b = r[g * 16:g * 16 + 8, _cols(u)], r[g * 16 + 8:g * 16 + 16, _cols(u)]
                spec[c, b0 + u, g * 24:g * 24 + 8, :] = a + b
                spec[c, b0 + u, g * 24 + 8:g * 24 + 16, :] = b
                spec[c, b0 + u, g * 24 + 16:g * 24 + 24, :] = a

    def inverse(i):
        inv = jnp.concatenate([_unpack(wp[NG, (u + 1) * C // 2:(u + 2) * C // 2, :]) for u in range(2)], axis=1)
        z = jnp.concatenate([_unpack(zb[c, i]) for c in range(NG)], axis=1)
        y = jnp.dot(inv, z, preferred_element_type=_F32)
        for c in range(NG):
            yb[c, pl.ds(pl.multiple_of(i * C, C), C), :] = y[:, _cols(c)]

    def permute_w(p):
        for n in range(NG):
            t = ws[:, pl.ds(pl.multiple_of(p * D + n * LANES, LANES), LANES)].astype(_F32).T
            for c in range(NG):
                wt32[c, _cols(n), :] = t[:, _cols(c)]
        for c in range(NG):
            for d in range(DH):
                rows = pl.ds(pl.multiple_of(p * (D // 2) + d * (H // 2), H // 2), H // 2)
                wp[c, rows, :] = _pack(wt32[c, pl.ds(d, H, stride=DH), :])

    def permute_wo(c):
        wt32[c] = wos[:, _cols(c)].astype(_F32)
        for d in range(DH):
            wp[c, (3 * D + d * H) // 2:(3 * D + (d + 1) * H) // 2, :] = _pack(wt32[c, pl.ds(d, H, stride=DH), :])

    def block_conv(c, r):
        r24 = pl.multiple_of(r * 24, 8)
        tok = pl.ds(pl.multiple_of(r * 8, 8), 8)
        cnt = 0
        prev = None
        for i0 in range(0, NB, TILE):
            ks = []
            for p in range(3):
                rows = pl.ds(r24 + 8 * p, 8)
                acc = [None] * TILE
                hw = {}
                for j0 in range(0, i0 + TILE, TILE):
                    need = {i - j for i in range(i0, i0 + TILE) for j in range(j0, j0 + TILE) if i >= j}
                    hw = {m: hw[m] if m in hw else spec[c, NB + m, rows, :] for m in sorted(need)}
                    for j in range(j0, j0 + TILE):
                        xj = spec[c, j, rows, :]
                        for i in range(max(i0, j), i0 + TILE):
                            t = xj * hw[i - j]
                            acc[i - i0] = t if acc[i - i0] is None else acc[i - i0] + t
                    cnt += 1
                    if cnt % PACE == 0:
                        for n, v in enumerate(acc):
                            spec[c, 2 * NB, pl.ds(pl.multiple_of(r * 8 + n * C // 2, 8), 8), :] = v
                ks.append(acc)
            for u in range(TILE):
                yr, yi = ks[0][u] - ks[1][u], ks[0][u] + ks[2][u]
                zr, zi = (yr, yi) if prev is None else (yr - prev[1], yi + prev[0])
                prev = yr, yi
                z = jnp.concatenate([zr, zi], axis=0)
                zb[c, i0 + u, tok, :] = _pack(z)

    scale = DH ** -0.5


    def weights(p):
        rows = pl.ds(pl.multiple_of(p * (D // 2), D // 2), D // 2)
        return jnp.concatenate([_unpack(wp[c, rows, :]) for c in range(NG)], axis=1)

    def project(n):
        i, p = n // 3, n % 3
        xb = xs[pl.ds(pl.multiple_of(i * TB, TB), TB), :]
        r = jax.lax.dot_general(xb, weights(p), _NT, preferred_element_type=_F32)
        for c in range(NG):
            qkv[p * NG + c, pl.ds(pl.multiple_of(HALO + i * TB, HALO), TB), :] = r[:, _cols(c)]

    def attend(s, u, masked):
        r0 = pl.multiple_of(HALO + s * TB + u * SUB, SUB)
        q = [qkv[c, pl.ds(r0, SUB), :] for c in range(NG)]
        logits = []
        for w in range(WIN):
            rows = pl.ds(r0 - DIL * w, SUB)
            p = q[0] * qkv[NG, rows, :]
            for c in range(1, NG):
                p = p + q[c] * qkv[NG + c, rows, :]
            logits.append(p)
        logits = [p + pltpu.roll(p, 2 * H, 1) for p in logits]
        yield
        logits = [p + pltpu.roll(p, H, 1) for p in logits]
        yield
        if masked and u * SUB < DIL * (WIN - 1):
            row = u * SUB + jax.lax.broadcasted_iota(jnp.int32, (SUB, LANES), 0)
            logits = [p if w == 0 else jnp.where(row >= DIL * w, p, -1e9 / scale)
                      for w, p in enumerate(logits)]
        m = _tree(jnp.maximum, logits)
        e = [jnp.exp2((l - m) * (scale * np.log2(np.e))) for l in logits]
        rden = 1.0 / _tree(jnp.add, e)
        for c in range(NG):
            acc = e[0] * qkv[2 * NG + c, pl.ds(r0, SUB), :]
            for w in range(1, WIN):
                acc = acc + e[w] * qkv[2 * NG + c, pl.ds(r0 - DIL * w, SUB), :]
            obuf[c, pl.ds(pl.multiple_of(s * (TB // 2) + u * (SUB // 2), SUB // 2), SUB // 2), :] = _pack(acc * rden)
        yield

    def out_copy(i):
        rows = pl.ds(pl.multiple_of(i * TB, TB), TB)
        return pltpu.make_async_copy(ob.at[rows, :], o_hbm.at[rows, :], sem_out.at[i])

    def out_proj(i):
        rows = pl.ds(pl.multiple_of(i * TB, TB), TB)
        half = pl.ds(pl.multiple_of(i * (TB // 2), TB // 2), TB // 2)
        o = jnp.concatenate([_unpack(obuf[c, half, :]) for c in range(NG)], axis=1)
        b = jnp.dot(o, weights(3), preferred_element_type=_F32)
        xf = [xs[rows, _cols(c)].astype(_F32) for c in range(NG)]
        gs = xf[0] * gvec[0:1, :]
        for c in range(1, NG):
            gs = gs + xf[c] * gvec[c:c + 1, :]
        g = jax.nn.sigmoid(jnp.sum(gs, axis=1, keepdims=True))
        for c in range(NG):
            bc = b[:, _cols(c)]
            ob[rows, _cols(c)] = (bc + g * (xf[c] * yb[c, rows, :] - bc)).astype(_BF16)
        out_copy(i).start()

    nstep = S // TB
    npos = NR // NQ

    def attention(s, masked=False):
        n = TB // SUB
        work = [attend(s, u, masked) for u in range(n)]
        next(work[0])
        for u in range(n):
            if u + 1 < n:
                next(work[u + 1])
            next(work[u])
            next(work[u])
        for u in range(TB // C):
            inverse(s * (TB // C) + u)

    def conv_step(c, q):
        for u in range(npos):
            block_conv(c, q * npos + u)

    @pl.loop(0, NG)
    def _(c):
        h_copy(c).wait()
        for q in range(NQ):
            forward_h(c, q)

    @pl.loop(0, 3)
    def _(p):
        w_copy(p).wait()
        permute_w(p)

    cp_x[0].wait()

    project(0)

    @pl.loop(0, NQ - 1)
    def _(q):
        for cp in kv_copies(q):
            cp.wait()

        @pl.when(q + 1 == 3)
        def _():
            cp_x[1].wait()

        project(q + 1)
        for c in range(NG):
            forward_kv(c, q)

    for cp in kv_copies(NQ - 1):
        cp.wait()
    for c in range(NG):
        forward_kv(c, NQ - 1)

    @pl.loop(0, NG * NQ)
    def _(n):
        @pl.when(NQ + n == 6)
        def _():
            cp_x[2].wait()
        project(NQ + n)
        conv_step(n // NQ, n % NQ)

    cp_wo.wait()
    attention(0, masked=True)
    for c in range(NG):
        permute_wo(c)

    @pl.loop(1, nstep)
    def _(s):
        out_proj(s - 1)
        attention(s)

    out_proj(nstep - 1)
    for i in range(nstep):
        out_copy(i).wait()


@jax.jit
def pallas_gated_mix__ssm_conv_h3__sliding_local_dilated__prompt_kernel(
    A_q: jax.Array,
    A_k: jax.Array,
    A_v: jax.Array,
    A_shift_k: jax.Array,
    A_ssm_k: jax.Array,
    A_ssm_D: jax.Array,
    B_x: jax.Array,
    B_wqkv: jax.Array,
    B_wo: jax.Array,
    gate_w: jax.Array,
):
    del B_x
    hbm = pl.BlockSpec(memory_space=pl.ANY)
    vmem = pl.BlockSpec(memory_space=pltpu.VMEM)
    V = pltpu.VMEM
    out = pl.pallas_call(
        _kernel,
        out_shape=jax.ShapeDtypeStruct((S, D), _BF16),
        in_specs=[hbm, hbm, hbm, vmem, hbm, vmem, hbm, hbm, vmem, vmem, vmem],
        out_specs=hbm,
        scratch_shapes=[
            V((S, D), _BF16),
            V((S, D), _BF16),
            V((S, D), _BF16),
            V((D, S), _BF16),
            V((D, 3 * D), _BF16),
            V((D, D), _BF16),
            V((NG, D, LANES), _F32),
            V((NG + 1, 4 * D // 2, LANES), _U32),
            V((3 * NG, HALO + S, LANES), _F32),
            V((NG, S // 2, LANES), _U32),
            V((NG, CHALO + S, LANES), _F32),
            V((NG, 8, LANES), _F32),
            V((NG, S, LANES), _F32),
            V((S, D), _BF16),
            V((NG, NB, C, LANES), _U32),
            V((NG, 2 * NB + 1, 3 * C, LANES), _F32),
            pltpu.SemaphoreType.DMA((NG + 2 * NQ + 7,)),
            pltpu.SemaphoreType.DMA((S // TB,)),
        ],
        compiler_params=pltpu.CompilerParams(vmem_limit_bytes=112 * 2**20),
    )(
        A_q.reshape(S, D), A_k.reshape(S, D), A_v.reshape(S, D), A_shift_k.T, A_ssm_k,
        A_ssm_D.reshape(NG, LANES), B_wqkv, B_wo, gate_w.reshape(NG, LANES),
        jnp.asarray(_FWD, _BF16), jnp.asarray(_INV, _BF16),
    )
    return out.reshape(1, S, D)
```
